```python
import os as _os
_os.environ.setdefault("JAX_PLATFORMS", "cpu")
import jax
import jax.numpy as jnp

def _softmax(x, axis=-1):
    return jax.nn.softmax(x, axis=axis)
def _gelu(x):
    return jax.nn.gelu(x, approximate=True)
def _silu(x):
    return jax.nn.silu(x)
def _sigmoid(x):
    return jax.nn.sigmoid(x)
def _layernorm(x, axis=-1, eps=1e-5):
    m = jnp.mean(x, axis=axis, keepdims=True)
    v = jnp.var(x, axis=axis, keepdims=True)
    return (x - m) / jnp.sqrt(v + eps)
def _scatter_add(tgt, idx, src, axis=0):
    return tgt.at[idx].add(src)
def _segment_sum(src, seg, n):
    return jax.ops.segment_sum(src, seg, n)
class _Rng:
    def __init__(self, key):
        self._k = key
    def _next(self):
        self._k, sub = jax.random.split(self._k)
        return sub
    def normal(self, shape):
        return jax.random.normal(self._next(), shape, dtype=jnp.bfloat16)
    def randint(self, lo, hi, shape):
        return jax.random.randint(self._next(), shape, lo, hi, dtype=jnp.int32)
    def uniform(self, shape, lo=0.0, hi=1.0):
        return jax.random.uniform(self._next(), shape, jnp.bfloat16, lo, hi)
    def permutation(self, n):
        return jax.random.permutation(self._next(), n)


kernel_name = 'concat_heads__gqa_block_cached__gqa_block_cached__near_ridge'

def setup_inputs():
    _rng = _Rng(jax.random.key(int.from_bytes(__import__("os").urandom(4), "little")))
    _w = (lambda a: (lambda t: t.astype(jnp.bfloat16) if jnp.issubdtype(t.dtype, jnp.floating) else t)(jnp.asarray(a)))
    def _A_setup():
        B, Sq, D = 16, 144, 448
        Hq, Hkv, Sk, Dh = 16, 8, 1024, 256
        assert Hq % Hkv == 0, (Hq, Hkv)
        return {
            "x": _w((lambda *s: _rng.normal(s) * 0.8)(B, Sq, D)),
            "k_cache": _w((lambda *s: _rng.normal(s) * 0.8)(B, Hkv, Sk, Dh)),
            "v_cache": _w((lambda *s: _rng.normal(s) * 0.05)(B, Hkv, Sk, Dh)),
            "wq": _w((lambda *s: _rng.normal(s) * 0.8)(D, Hq * Dh) * (D ** -0.5)),
            "wo": _w((lambda *s: _rng.normal(s) * 0.05)(Hq * Dh, D) * ((Hq * Dh) ** -0.5)),
        }
    _A_in = _A_setup()

    def _B_setup():
        B, Sq, D = 16, 144, 448
        Hq, Hkv, Sk, Dh = 16, 8, 1024, 256
        assert Hq % Hkv == 0, (Hq, Hkv)
        return {
            "x": _w((lambda *s: _rng.normal(s) * 0.8)(B, Sq, D)),
            "k_cache": _w((lambda *s: _rng.normal(s) * 0.8)(B, Hkv, Sk, Dh)),
            "v_cache": _w((lambda *s: _rng.normal(s) * 0.05)(B, Hkv, Sk, Dh)),
            "wq": _w((lambda *s: _rng.normal(s) * 0.8)(D, Hq * Dh) * (D ** -0.5)),
            "wo": _w((lambda *s: _rng.normal(s) * 0.05)(Hq * Dh, D) * ((Hq * Dh) ** -0.5)),
        }
    _B_in = _B_setup()

    return {
        "A_x": _A_in["x"],
        "A_k_cache": _A_in["k_cache"],
        "A_v_cache": _A_in["v_cache"],
        "A_wq": _A_in["wq"],
        "A_wo": _A_in["wo"],
        "B_x": _B_in["x"],
        "B_k_cache": _B_in["k_cache"],
        "B_v_cache": _B_in["v_cache"],
        "B_wq": _B_in["wq"],
        "B_wo": _B_in["wo"],
    }

def reference(A_x, A_k_cache, A_v_cache, A_wq, A_wo, B_x, B_k_cache, B_v_cache, B_wq, B_wo):
    def _A_ref(x, k_cache, v_cache, wq, wo):
        B, Sq, D = x.shape
        Hq, Dh = 16, 256
        Hkv = k_cache.shape[1]
        rep = Hq // Hkv
        q = (lambda x, *d: x.transpose(*d))((x @ wq).reshape(B, Sq, Hq, Dh), 0, 2, 1, 3)
        k = jnp.repeat(k_cache, rep, axis=1)
        v = jnp.repeat(v_cache, rep, axis=1)
        scores = jnp.einsum("bhqd,bhkd->bhqk", q, k) * (Dh ** -0.5)
        p = _softmax(scores, axis=-1)
        o = jnp.einsum("bhqk,bhkd->bhqd", p, v)
        return (lambda x, *d: x.transpose(*d))(o, 0, 2, 1, 3).reshape(B, Sq, Hq * Dh) @ wo

    def _B_ref(x, k_cache, v_cache, wq, wo):
        B, Sq, D = x.shape
        Hq, Dh = 16, 256
        Hkv = k_cache.shape[1]
        rep = Hq // Hkv
        q = (lambda x, *d: x.transpose(*d))((x @ wq).reshape(B, Sq, Hq, Dh), 0, 2, 1, 3)
        k = jnp.repeat(k_cache, rep, axis=1)
        v = jnp.repeat(v_cache, rep, axis=1)
        scores = jnp.einsum("bhqd,bhkd->bhqk", q, k) * (Dh ** -0.5)
        p = _softmax(scores, axis=-1)
        o = jnp.einsum("bhqk,bhkd->bhqd", p, v)
        return (lambda x, *d: x.transpose(*d))(o, 0, 2, 1, 3).reshape(B, Sq, Hq * Dh) @ wo

    a = _A_ref(A_x, A_k_cache, A_v_cache, A_wq, A_wo)
    b = _B_ref(B_x, B_k_cache, B_v_cache, B_wq, B_wo)
    return jnp.concatenate([a, b], axis=-1)
```

```python
import jax
import jax.numpy as jnp
from jax import lax
import jax.experimental.pallas as pl
import jax.experimental.pallas.tpu as pltpu

B, SQ, D = 16, 144, 448
HQ, HKV, SK, DH = 16, 8, 1024, 256
REP = HQ // HKV
GW = REP * DH
MQ = REP * SQ

NB = 8
NG = 2
UNITS = NB * NG
TOK = NB * SQ
TT = 128
NTILE = TOK // TT
NGP = HKV // NG
NIT = (B // NB) * 2 * NGP
DEFER = 2

OFF = (D // 128) * 128
WIN = 2 * D - OFF
EDGE = D - OFF

QB = 4
QPRE = 4
QL = 3
RC = 16
LANES = 2

F32 = jnp.float32
BF16 = jnp.bfloat16
U32 = jnp.uint32
NT = (((1,), (1,)), ((), ()))
LOG2E = 1.4426950408889634
QSCALE = DH ** -0.5 * LOG2E


def _kernel(xa_h, ka_h, va_h, wqa_h, woa_h, xb_h, kb_h, vb_h, wqb_h, wob_h, o_h,
            x_v, wq_v, wo_v, q_v, kv_v, acc, edge, o_v, p0_v, p1_v, a0_v, a1_v,
            kv_sem, x_sem, wq_sem, wo_sem, o_sem):
    x_h = (xa_h, xb_h)
    k_h = (ka_h, kb_h)
    v_h = (va_h, vb_h)
    wq_h = (wqa_h, wqb_h)
    wo_h = (woa_h, wob_h)
    p_v = (p0_v, p1_v)
    a_v = (a0_v, a1_v)

    def start(copies):
        for c in copies:
            c.start()

    def wait(copies):
        for c in copies:
            c.wait()

    def coords(it):
        return it // (2 * NGP), (it // NGP) % 2, it % NGP

    def kv_copies(it, r):
        bg, _, gp = coords(it)
        slot = it % 2
        return [pltpu.make_async_copy(src[r].at[pl.ds(bg * NB, NB), pl.ds(gp * NG, NG)],
                                      kv_v.at[slot, j], kv_sem.at[slot])
                for j, src in enumerate((k_h, v_h))]

    def kv_wait(it):
        pltpu.make_async_copy(kv_v.at[it % 2], kv_v.at[it % 2], kv_sem.at[it % 2]).wait()

    def x_copy(r, lo, hi, j):
        rows = pl.ds(lo * SQ, (hi - lo) * SQ)
        return pltpu.make_async_copy(x_h[r].at[rows], x_v.at[r, rows], x_sem.at[j])

    def wq_copy(g, r):
        return pltpu.make_async_copy(wq_h[r].at[:, pl.ds(g * GW, GW)], wq_v.at[r, g], wq_sem.at[r, g])

    def wo_copy(gp, r):
        return pltpu.make_async_copy(wo_h[r].at[:, pl.ds(gp * NG * GW, NG * GW)], wo_v.at[r, gp],
                                     wo_sem.at[r, gp])

    def o_copy(bg, r, t0=0, t1=NTILE, j=0):
        rows = pl.ds(bg * TOK + t0 * TT, (t1 - t0) * TT)
        sem = o_sem.at[2 * bg + r + j]
        if r == 0:
            return pltpu.make_async_copy(o_v.at[0, rows, pl.ds(0, OFF)], o_h.at[rows, pl.ds(0, OFF)], sem)
        return pltpu.make_async_copy(o_v.at[1, rows], o_h.at[rows, pl.ds(OFF, WIN)], sem)

    def qproj(g, r, lo, hi):
        for b0 in range(lo, hi, QB):
            q = jnp.dot(x_v[r, b0 * SQ:(b0 + QB) * SQ, :], wq_v[r, g], preferred_element_type=F32)
            q = (q * QSCALE).astype(BF16)
            for n in range(QB):
                for h in range(REP):
                    q_v[g, r, b0 + n, h * SQ // 2:(h + 1) * SQ // 2, :] = pltpu.bitcast(
                        q[n * SQ:(n + 1) * SQ, h * DH:(h + 1) * DH], U32)

    c0 = [wq_copy(0, 0), x_copy(0, 0, QB, 0)]
    c1 = [x_copy(0, QB, 2 * QB, 1)]
    c2 = [x_copy(0, 2 * QB, B, 2)]
    c3 = [wq_copy(g, 0) for g in range(1, QPRE)]
    c4 = ([wq_copy(g, 0) for g in range(QPRE, HKV)] + [x_copy(1, 0, B, 3)]
          + [wq_copy(g, 1) for g in range(HKV)])
    c5 = [wo_copy(gp, r) for gp in range(NGP) for r in range(2)]
    start(c0)
    start(c1)
    for t in range(NTILE):
        acc[t] = jnp.zeros((D, TT), F32)
        edge[t] = jnp.zeros((EDGE, TT), F32)
    wait(c0)
    start(c2)
    qproj(0, 0, 0, QB)
    wait(c1)
    start(c3)
    qproj(0, 0, QB, 2 * QB)
    wait(c2)
    start(c4)
    qproj(0, 0, 2 * QB, B)
    wait(c3)
    for g in range(1, QPRE):
        qproj(g, 0, 0, B)

    def q_step(j, carry):
        @pl.when(j == 0)
        def _():
            wait(c4)
            start(kv_copies(0, coords(0)[1]))

        @pl.when(j == 1)
        def _():
            start(c5)

        @pl.when(j == 2)
        def _():
            start(kv_copies(1, coords(1)[1]))

        for i in range(QL):
            blk = QPRE + j * QL + i
            qproj(blk % HKV, blk // HKV, 0, B)
        return carry

    lax.fori_loop(0, (2 * HKV - QPRE) // QL, q_step, 0)
    wait(c5)

    def emit(it, t, y):
        bg, r, _ = coords(it)
        is_a = r == 0
        e = jnp.where(is_a, y[OFF:], edge[t])
        edge[t] = e
        yy = jnp.where(is_a, jnp.concatenate([y, e], axis=0), jnp.concatenate([e, y], axis=0))
        o_v[r, pl.ds(pl.multiple_of(bg * TOK + t * TT, TT), TT), :] = yy.T.astype(BF16)

    def body(it):
        bg, r, gp = coords(it)
        slot = it % 2
        scores = {}
        inv_sum = {}
        partial = {}

        def qk(u):
            n, gg = divmod(u, NG)
            for h in range(REP):
                q = pltpu.bitcast(
                    q_v[gp * NG + gg, r, bg * NB + n, h * SQ // 2:(h + 1) * SQ // 2, :], BF16)
                scores[u, h] = lax.dot_general(q, kv_v[slot, 0, n, gg], NT, preferred_element_type=F32)

        def softmax(u):
            sums = []
            for c in range(MQ // RC):
                h, r0 = divmod(c * RC, SQ)
                s = scores[u, h][r0:r0 + RC]
                m = jnp.max(s, axis=-1, keepdims=True)
                if c >= LANES:
                    m = jnp.where(sums[c - LANES] < -1.0, 0.0, m)
                p = jnp.exp2(s - m)
                sums.append(jnp.sum(p, axis=-1, keepdims=True))
                inv_sum[u, c] = 1.0 / sums[c]
                p_v[u % 2][c * RC // 2:(c + 1) * RC // 2, :] = pltpu.bitcast(p.astype(BF16), U32)

        def pv(u):
            n, gg = divmod(u, NG)
            p = pltpu.bitcast(p_v[u % 2][...], BF16)
            inv = jnp.concatenate([inv_sum[u, c] for c in range(MQ // RC)], axis=0)
            o = jnp.dot(p, kv_v[slot, 1, n, gg], preferred_element_type=F32)
            o = (o * inv).astype(BF16)
            for h in range(REP):
                a_v[gg][n * SQ // 2:(n + 1) * SQ // 2, h * DH:(h + 1) * DH] = pltpu.bitcast(
                    o[h * SQ:(h + 1) * SQ], U32)

        def oproj(u):
            n, gg = divmod(u, NG)
            for t in range(NTILE):
                if ((t + 1) * TT - 1) // SQ != n:
                    continue
                o = pltpu.bitcast(a_v[gg][t * TT // 2:(t + 1) * TT // 2, :], BF16)
                y = lax.dot_general(wo_v[r, gp, :, gg * GW:(gg + 1) * GW], o, NT,
                                    preferred_element_type=F32)
                if gg == 0:
                    partial[t] = y
                    continue
                y = y + jnp.where(gp == 0, 0.0, acc[t]) + partial[t]
                acc[t] = y
                if t < NTILE - DEFER:
                    emit(it, t, y)

        for t in range(NTILE - DEFER, NTILE):
            emit(jnp.maximum(it - 1, 0), t, acc[t])
        qk(0)
        qk(1)
        softmax(0)
        for u in range(UNITS):
            pv(u)
            if u >= 1:
                oproj(u - 1)
            if u + 2 < UNITS:
                qk(u + 2)
            if u + 1 < UNITS:
                softmax(u + 1)
        oproj(UNITS - 1)

    def step(it, carry):
        kv_wait(it)
        body(it)
        for r in range(2):
            @pl.when(jnp.logical_and(it + 2 < NIT, coords(it + 2)[1] == r))
            def _():
                start(kv_copies(it + 2, r))
        for j in range(NIT // NGP - 1):
            @pl.when(it == (j + 1) * NGP)
            def _():
                o_copy(j // 2, j % 2).start()
        return carry

    lax.fori_loop(0, NIT, step, 0)

    last_bg = B // NB - 1
    tail = [o_copy(last_bg, 1, 0, NTILE - DEFER, 0), o_copy(last_bg, 1, NTILE - DEFER, NTILE, 1)]
    tail[0].start()
    for t in range(NTILE - DEFER, NTILE):
        emit(NIT - 1, t, acc[t])
    tail[1].start()
    wait([o_copy(j // 2, j % 2) for j in range(NIT // NGP - 1)] + tail)


@jax.jit
def pallas_concat_heads__gqa_block_cached__gqa_block_cached__near_ridge_kernel(
    A_x: jax.Array,
    A_k_cache: jax.Array,
    A_v_cache: jax.Array,
    A_wq: jax.Array,
    A_wo: jax.Array,
    B_x: jax.Array,
    B_k_cache: jax.Array,
    B_v_cache: jax.Array,
    B_wq: jax.Array,
    B_wo: jax.Array,
):
    hbm = pl.BlockSpec(memory_space=pltpu.HBM)
    out = pl.pallas_call(
        _kernel,
        in_specs=[hbm] * 10,
        out_specs=hbm,
        out_shape=jax.ShapeDtypeStruct((B * SQ, 2 * D), BF16),
        scratch_shapes=[
            pltpu.VMEM((2, B * SQ, D), BF16),
            pltpu.VMEM((2, HKV, D, GW), BF16),
            pltpu.VMEM((2, NGP, D, NG * GW), BF16),
            pltpu.VMEM((HKV, 2, B, MQ // 2, DH), U32),
            pltpu.VMEM((2, 2, NB, NG, SK, DH), BF16),
            pltpu.VMEM((NTILE, D, TT), F32),
            pltpu.VMEM((NTILE, EDGE, TT), F32),
            pltpu.VMEM((2, B * SQ, WIN), BF16),
            pltpu.VMEM((MQ // 2, SK), U32),
            pltpu.VMEM((MQ // 2, SK), U32),
            pltpu.VMEM((TOK // 2, GW), U32),
            pltpu.VMEM((TOK // 2, GW), U32),
            pltpu.SemaphoreType.DMA((2,)),
            pltpu.SemaphoreType.DMA((4,)),
            pltpu.SemaphoreType.DMA((2, HKV)),
            pltpu.SemaphoreType.DMA((2, NGP)),
            pltpu.SemaphoreType.DMA((NIT // NGP + 1,)),
        ],
        compiler_params=pltpu.CompilerParams(
            vmem_limit_bytes=120 * 1024 * 1024, disable_bounds_checks=True),
    )(A_x.reshape(B * SQ, D), A_k_cache, A_v_cache, A_wq, A_wo.T,
      B_x.reshape(B * SQ, D), B_k_cache, B_v_cache, B_wq, B_wo.T)
    return out.reshape(B, SQ, 2 * D)
```

```python
import jax
import jax.numpy as jnp
from jax import lax
import jax.experimental.pallas as pl
import jax.experimental.pallas.tpu as pltpu

B, SQ, D = 16, 144, 448
HQ, HKV, SK, DH = 16, 8, 1024, 256
REP = HQ // HKV
GW = REP * DH
MQ = REP * SQ

NB = 8
NG = 2
UNITS = NB * NG
TOK = NB * SQ
TT = 128
NTILE = TOK // TT
NGP = HKV // NG
NIT = (B // NB) * 2 * NGP
DEFER = 2

OFF = (D // 128) * 128
WIN = 2 * D - OFF
EDGE = D - OFF

QB = 4
QPRE = 4
QL = 3
RC = 16
LANES = 2

F32 = jnp.float32
BF16 = jnp.bfloat16
U32 = jnp.uint32
NT = (((1,), (1,)), ((), ()))
LOG2E = 1.4426950408889634
QSCALE = DH ** -0.5 * LOG2E


def _kernel(xa_h, ka_h, va_h, wqa_h, woa_h, xb_h, kb_h, vb_h, wqb_h, wob_h, o_h,
            x_v, wq_v, wo_v, q_v, kv_v, acc, edge, o_v, p0_v, p1_v, a0_v, a1_v,
            kv_sem, in_sem, o_sem):
    x_h = (xa_h, xb_h)
    k_h = (ka_h, kb_h)
    v_h = (va_h, vb_h)
    wq_h = (wqa_h, wqb_h)
    wo_h = (woa_h, wob_h)
    p_v = (p0_v, p1_v)
    a_v = (a0_v, a1_v)

    def start(copies):
        for c in copies:
            c.start()

    def wait(copies):
        for c in copies:
            c.wait()

    def coords(it):
        return it // (2 * NGP), (it // NGP) % 2, it % NGP

    def kv_copies(it, r):
        bg, _, gp = coords(it)
        slot = it % 2
        return [pltpu.make_async_copy(src[r].at[pl.ds(bg * NB, NB), pl.ds(gp * NG, NG)],
                                      kv_v.at[slot, j], kv_sem.at[slot])
                for j, src in enumerate((k_h, v_h))]

    def kv_wait(it):
        pltpu.make_async_copy(kv_v.at[it % 2], kv_v.at[it % 2], kv_sem.at[it % 2]).wait()

    def x_copy(r, lo, hi, group):
        rows = pl.ds(lo * SQ, (hi - lo) * SQ)
        return pltpu.make_async_copy(x_h[r].at[rows], x_v.at[r, rows], in_sem.at[group])

    def wq_copy(g, r, group):
        return pltpu.make_async_copy(wq_h[r].at[:, pl.ds(g * GW, GW)], wq_v.at[r, g], in_sem.at[group])

    def wo_copy(gp, r, group):
        return pltpu.make_async_copy(wo_h[r].at[:, pl.ds(gp * NG * GW, NG * GW)], wo_v.at[r, gp],
                                     in_sem.at[group])

    def o_copy(bg, r, t0=0, t1=NTILE):
        rows = pl.ds(bg * TOK + t0 * TT, (t1 - t0) * TT)
        if r == 0:
            return pltpu.make_async_copy(o_v.at[0, rows, pl.ds(0, OFF)], o_h.at[rows, pl.ds(0, OFF)],
                                         o_sem.at[0])
        return pltpu.make_async_copy(o_v.at[1, rows], o_h.at[rows, pl.ds(OFF, WIN)], o_sem.at[0])

    def qproj(g, r, lo, hi):
        for b0 in range(lo, hi, QB):
            q = jnp.dot(x_v[r, b0 * SQ:(b0 + QB) * SQ, :], wq_v[r, g], preferred_element_type=F32)
            q = (q * QSCALE).astype(BF16)
            for n in range(QB):
                for h in range(REP):
                    q_v[g, r, b0 + n, h * SQ // 2:(h + 1) * SQ // 2, :] = pltpu.bitcast(
                        q[n * SQ:(n + 1) * SQ, h * DH:(h + 1) * DH], U32)

    c0 = [wq_copy(0, 0, 0), x_copy(0, 0, QB, 0)]
    c1 = [x_copy(0, QB, 2 * QB, 1)]
    c2 = [x_copy(0, 2 * QB, B, 2)]
    c3 = [wq_copy(g, 0, 3) for g in range(1, QPRE)]
    c4 = ([wq_copy(g, 0, 4) for g in range(QPRE, HKV)] + [x_copy(1, 0, B, 4)]
          + [wq_copy(g, 1, 4) for g in range(HKV)])
    c5 = [wo_copy(gp, r, 5) for gp in range(NGP) for r in range(2)]
    start(c0)
    start(c1)
    for t in range(NTILE):
        acc[t] = jnp.zeros((D, TT), F32)
        edge[t] = jnp.zeros((EDGE, TT), F32)
    wait(c0)
    start(c2)
    qproj(0, 0, 0, QB)
    wait(c1)
    start(c3)
    qproj(0, 0, QB, 2 * QB)
    wait(c2)
    start(c4)
    qproj(0, 0, 2 * QB, B)
    wait(c3)
    for g in range(1, QPRE):
        qproj(g, 0, 0, B)

    def q_step(j, carry):
        @pl.when(j == 0)
        def _():
            wait(c4)
            start(kv_copies(0, coords(0)[1]))

        @pl.when(j == 1)
        def _():
            start(c5)

        @pl.when(j == 2)
        def _():
            start(kv_copies(1, coords(1)[1]))

        for i in range(QL):
            blk = QPRE + j * QL + i
            qproj(blk % HKV, blk // HKV, 0, B)
        return carry

    lax.fori_loop(0, (2 * HKV - QPRE) // QL, q_step, 0)
    wait(c5)

    def emit(it, t, y):
        bg, r, _ = coords(it)
        is_a = r == 0
        e = jnp.where(is_a, y[OFF:], edge[t])
        edge[t] = e
        yy = jnp.where(is_a, jnp.concatenate([y, e], axis=0), jnp.concatenate([e, y], axis=0))
        o_v[r, pl.ds(pl.multiple_of(bg * TOK + t * TT, TT), TT), :] = yy.T.astype(BF16)

    def body(it):
        bg, r, gp = coords(it)
        slot = it % 2
        scores = {}
        inv_sum = {}
        partial = {}

        def qk(u, h):
            n, gg = divmod(u, NG)
            q = pltpu.bitcast(
                q_v[gp * NG + gg, r, bg * NB + n, h * SQ // 2:(h + 1) * SQ // 2, :], BF16)
            scores[u, h] = lax.dot_general(q, kv_v[slot, 0, n, gg], NT, preferred_element_type=F32)

        def softmax(u):
            sums = []
            for c in range(MQ // RC):
                h, r0 = divmod(c * RC, SQ)
                s = scores[u, h][r0:r0 + RC]
                m = jnp.max(s, axis=-1, keepdims=True)
                if c >= LANES:
                    m = jnp.where(sums[c - LANES] < -1.0, 0.0, m)
                p = jnp.exp2(s - m)
                sums.append(jnp.sum(p, axis=-1, keepdims=True))
                inv_sum[u, c] = 1.0 / sums[c]
                p_v[u % 2][c * RC // 2:(c + 1) * RC // 2, :] = pltpu.bitcast(p.astype(BF16), U32)

        def pv(u):
            n, gg = divmod(u, NG)
            p = pltpu.bitcast(p_v[u % 2][...], BF16)
            inv = jnp.concatenate([inv_sum[u, c] for c in range(MQ // RC)], axis=0)
            o = jnp.dot(p, kv_v[slot, 1, n, gg], preferred_element_type=F32)
            o = (o * inv).astype(BF16)
            for h in range(REP):
                a_v[gg][n * SQ // 2:(n + 1) * SQ // 2, h * DH:(h + 1) * DH] = pltpu.bitcast(
                    o[h * SQ:(h + 1) * SQ], U32)

        def oproj(u):
            n, gg = divmod(u, NG)
            for t in range(NTILE):
                if ((t + 1) * TT - 1) // SQ != n:
                    continue
                o = pltpu.bitcast(a_v[gg][t * TT // 2:(t + 1) * TT // 2, :], BF16)
                y = lax.dot_general(wo_v[r, gp, :, gg * GW:(gg + 1) * GW], o, NT,
                                    preferred_element_type=F32)
                if gg == 0:
                    partial[t] = y
                    continue
                y = y + jnp.where(gp == 0, 0.0, acc[t]) + partial[t]
                acc[t] = y
                if t < NTILE - DEFER:
                    emit(it, t, y)

        for t in range(NTILE - DEFER, NTILE):
            emit(jnp.maximum(it - 1, 0), t, acc[t])
        for u in range(2):
            for h in range(REP):
                qk(u, h)
        softmax(0)
        for u in range(UNITS):
            if u + 2 < UNITS:
                qk(u + 2, 0)
            pv(u)
            if u >= 1:
                oproj(u - 1)
            if u + 2 < UNITS:
                qk(u + 2, 1)
            if u + 1 < UNITS:
                softmax(u + 1)
        oproj(UNITS - 1)

    def step(it, carry):
        kv_wait(it)
        body(it)
        for r in range(2):
            @pl.when(jnp.logical_and(it + 2 < NIT, coords(it + 2)[1] == r))
            def _():
                start(kv_copies(it + 2, r))
        for j in range(NIT // NGP - 1):
            @pl.when(it == (j + 1) * NGP)
            def _():
                o_copy(j // 2, j % 2).start()
        return carry

    lax.fori_loop(0, NIT, step, 0)

    last_bg = B // NB - 1
    tail = [o_copy(last_bg, 1, 0, NTILE - DEFER), o_copy(last_bg, 1, NTILE - DEFER, NTILE)]
    tail[0].start()
    for t in range(NTILE - DEFER, NTILE):
        emit(NIT - 1, t, acc[t])
    tail[1].start()
    wait([o_copy(j // 2, j % 2) for j in range(NIT // NGP - 1)] + tail)


@jax.jit
def pallas_concat_heads__gqa_block_cached__gqa_block_cached__near_ridge_kernel(
    A_x: jax.Array,
    A_k_cache: jax.Array,
    A_v_cache: jax.Array,
    A_wq: jax.Array,
    A_wo: jax.Array,
    B_x: jax.Array,
    B_k_cache: jax.Array,
    B_v_cache: jax.Array,
    B_wq: jax.Array,
    B_wo: jax.Array,
):
    hbm = pl.BlockSpec(memory_space=pltpu.HBM)
    out = pl.pallas_call(
        _kernel,
        in_specs=[hbm] * 10,
        out_specs=hbm,
        out_shape=jax.ShapeDtypeStruct((B * SQ, 2 * D), BF16),
        scratch_shapes=[
            pltpu.VMEM((2, B * SQ, D), BF16),
            pltpu.VMEM((2, HKV, D, GW), BF16),
            pltpu.VMEM((2, NGP, D, NG * GW), BF16),
            pltpu.VMEM((HKV, 2, B, MQ // 2, DH), U32),
            pltpu.VMEM((2, 2, NB, NG, SK, DH), BF16),
            pltpu.VMEM((NTILE, D, TT), F32),
            pltpu.VMEM((NTILE, EDGE, TT), F32),
            pltpu.VMEM((2, B * SQ, WIN), BF16),
            pltpu.VMEM((MQ // 2, SK), U32),
            pltpu.VMEM((MQ // 2, SK), U32),
            pltpu.VMEM((TOK // 2, GW), U32),
            pltpu.VMEM((TOK // 2, GW), U32),
            pltpu.SemaphoreType.DMA((2,)),
            pltpu.SemaphoreType.DMA((6,)),
            pltpu.SemaphoreType.DMA((1,)),
        ],
        compiler_params=pltpu.CompilerParams(
            vmem_limit_bytes=120 * 1024 * 1024, disable_bounds_checks=True),
    )(A_x.reshape(B * SQ, D), A_k_cache, A_v_cache, A_wq, A_wo.T,
      B_x.reshape(B * SQ, D), B_k_cache, B_v_cache, B_wq, B_wo.T)
    return out.reshape(B, SQ, 2 * D)
```

```python
import jax
import jax.numpy as jnp
from jax import lax
import jax.experimental.pallas as pl
import jax.experimental.pallas.tpu as pltpu

B, SQ, D = 16, 144, 448
HQ, HKV, SK, DH = 16, 8, 1024, 256
REP = HQ // HKV
GW = REP * DH
MQ = REP * SQ

NB = 8
NG = 2
UNITS = NB * NG
TOK = NB * SQ
TT = 128
NTILE = TOK // TT
NGP = HKV // NG
NIT = (B // NB) * 2 * NGP
DEFER = 2

OFF = (D // 128) * 128
WIN = 2 * D - OFF
EDGE = D - OFF

QB = 4
QPRE = 4
QL = 3
RC = 16

F32 = jnp.float32
BF16 = jnp.bfloat16
U32 = jnp.uint32
NT = (((1,), (1,)), ((), ()))
LOG2E = 1.4426950408889634
QSCALE = DH ** -0.5 * LOG2E


def _kernel(xa_h, ka_h, va_h, wqa_h, woa_h, xb_h, kb_h, vb_h, wqb_h, wob_h, o_h,
            x_v, wq_v, wo_v, q_v, kv_v, acc, edge, o_v, p0_v, p1_v, a0_v, a1_v,
            kv_sem, in_sem, o_sem):
    x_h = (xa_h, xb_h)
    k_h = (ka_h, kb_h)
    v_h = (va_h, vb_h)
    wq_h = (wqa_h, wqb_h)
    wo_h = (woa_h, wob_h)
    p_v = (p0_v, p1_v)
    a_v = (a0_v, a1_v)

    def start(copies):
        for c in copies:
            c.start()

    def wait(copies):
        for c in copies:
            c.wait()

    def coords(it):
        return it // (2 * NGP), (it // NGP) % 2, it % NGP

    def kv_copies(it, r):
        bg, _, gp = coords(it)
        slot = it % 2
        return [pltpu.make_async_copy(src[r].at[pl.ds(bg * NB, NB), pl.ds(gp * NG, NG)],
                                      kv_v.at[slot, j], kv_sem.at[slot])
                for j, src in enumerate((k_h, v_h))]

    def kv_wait(it):
        pltpu.make_async_copy(kv_v.at[it % 2], kv_v.at[it % 2], kv_sem.at[it % 2]).wait()

    def x_copy(r, lo, hi, group):
        rows = pl.ds(lo * SQ, (hi - lo) * SQ)
        return pltpu.make_async_copy(x_h[r].at[rows], x_v.at[r, rows], in_sem.at[group])

    def wq_copy(g, r, group):
        return pltpu.make_async_copy(wq_h[r].at[:, pl.ds(g * GW, GW)], wq_v.at[r, g], in_sem.at[group])

    def wo_copy(gp, r, group):
        return pltpu.make_async_copy(wo_h[r].at[:, pl.ds(gp * NG * GW, NG * GW)], wo_v.at[r, gp],
                                     in_sem.at[group])

    def o_copy(bg, r, t0=0, t1=NTILE):
        rows = pl.ds(bg * TOK + t0 * TT, (t1 - t0) * TT)
        if r == 0:
            return pltpu.make_async_copy(o_v.at[0, rows, pl.ds(0, OFF)], o_h.at[rows, pl.ds(0, OFF)],
                                         o_sem.at[0])
        return pltpu.make_async_copy(o_v.at[1, rows], o_h.at[rows, pl.ds(OFF, WIN)], o_sem.at[0])

    def qproj(g, r, lo, hi):
        for b0 in range(lo, hi, QB):
            q = jnp.dot(x_v[r, b0 * SQ:(b0 + QB) * SQ, :], wq_v[r, g], preferred_element_type=F32)
            q = (q * QSCALE).astype(BF16)
            for n in range(QB):
                for h in range(REP):
                    q_v[g, r, b0 + n, h * SQ // 2:(h + 1) * SQ // 2, :] = pltpu.bitcast(
                        q[n * SQ:(n + 1) * SQ, h * DH:(h + 1) * DH], U32)

    c0 = [wq_copy(0, 0, 0), x_copy(0, 0, QB, 0)]
    c1 = [x_copy(0, QB, 2 * QB, 1)]
    c2 = [x_copy(0, 2 * QB, B, 2)]
    c3 = [wq_copy(g, 0, 3) for g in range(1, QPRE)]
    c4 = ([wq_copy(g, 0, 4) for g in range(QPRE, HKV)] + [x_copy(1, 0, B, 4)]
          + [wq_copy(g, 1, 4) for g in range(HKV)])
    c5 = [wo_copy(gp, r, 5) for gp in range(NGP) for r in range(2)]
    start(c0)
    start(c1)
    for t in range(NTILE):
        acc[t] = jnp.zeros((D, TT), F32)
        edge[t] = jnp.zeros((EDGE, TT), F32)
    wait(c0)
    start(c2)
    qproj(0, 0, 0, QB)
    wait(c1)
    start(c3)
    qproj(0, 0, QB, 2 * QB)
    wait(c2)
    start(c4)
    qproj(0, 0, 2 * QB, B)
    wait(c3)
    for g in range(1, QPRE):
        qproj(g, 0, 0, B)

    def q_step(j, carry):
        @pl.when(j == 0)
        def _():
            wait(c4)
            start(kv_copies(0, coords(0)[1]))

        @pl.when(j == 1)
        def _():
            start(c5)

        @pl.when(j == 2)
        def _():
            start(kv_copies(1, coords(1)[1]))

        for i in range(QL):
            blk = QPRE + j * QL + i
            qproj(blk % HKV, blk // HKV, 0, B)
        return carry

    lax.fori_loop(0, (2 * HKV - QPRE) // QL, q_step, 0)
    wait(c5)

    def emit(it, t, y):
        bg, r, _ = coords(it)
        is_a = r == 0
        e = jnp.where(is_a, y[OFF:], edge[t])
        edge[t] = e
        yy = jnp.where(is_a, jnp.concatenate([y, e], axis=0), jnp.concatenate([e, y], axis=0))
        o_v[r, pl.ds(pl.multiple_of(bg * TOK + t * TT, TT), TT), :] = yy.T.astype(BF16)

    def body(it):
        bg, r, gp = coords(it)
        slot = it % 2
        scores = {}
        inv_sum = {}
        partial = {}

        def qk(u, h):
            n, gg = divmod(u, NG)
            q = pltpu.bitcast(
                q_v[gp * NG + gg, r, bg * NB + n, h * SQ // 2:(h + 1) * SQ // 2, :], BF16)
            scores[u, h] = lax.dot_general(q, kv_v[slot, 0, n, gg], NT, preferred_element_type=F32)

        def softmax(u):
            for h in range(REP):
                row_sum = None
                for c in range(SQ // RC):
                    s = scores[u, h][c * RC:(c + 1) * RC]
                    m = jnp.max(s, axis=-1, keepdims=True)
                    if row_sum is not None:
                        m = jnp.maximum(m, jnp.where(row_sum < 0.0, m, -jnp.inf))
                    p = jnp.exp2(s - m)
                    row_sum = jnp.sum(p, axis=-1, keepdims=True)
                    inv_sum.setdefault(u, []).append(1.0 / row_sum)
                    r0 = (h * SQ + c * RC) // 2
                    p_v[u % 2][r0:r0 + RC // 2, :] = pltpu.bitcast(p.astype(BF16), U32)

        def pv(u):
            n, gg = divmod(u, NG)
            p = pltpu.bitcast(p_v[u % 2][...], BF16)
            inv = jnp.concatenate(inv_sum[u], axis=0)
            o = jnp.dot(p, kv_v[slot, 1, n, gg], preferred_element_type=F32)
            o = (o * inv).astype(BF16)
            for h in range(REP):
                a_v[gg][n * SQ // 2:(n + 1) * SQ // 2, h * DH:(h + 1) * DH] = pltpu.bitcast(
                    o[h * SQ:(h + 1) * SQ], U32)

        def oproj(u):
            n, gg = divmod(u, NG)
            for t in range(NTILE):
                if ((t + 1) * TT - 1) // SQ != n:
                    continue
                o = pltpu.bitcast(a_v[gg][t * TT // 2:(t + 1) * TT // 2, :], BF16)
                y = lax.dot_general(wo_v[r, gp, :, gg * GW:(gg + 1) * GW], o, NT,
                                    preferred_element_type=F32)
                if gg == 0:
                    partial[t] = y + jnp.where(gp == 0, 0.0, acc[t])
                    continue
                y = y + partial[t]
                acc[t] = y
                if t < NTILE - DEFER:
                    emit(it, t, y)

        for t in range(NTILE - DEFER, NTILE):
            emit(jnp.maximum(it - 1, 0), t, acc[t])
        for u in range(2):
            for h in range(REP):
                qk(u, h)
        softmax(0)
        for u in range(UNITS):
            if u + 2 < UNITS:
                qk(u + 2, 0)
            pv(u)
            if u >= 1:
                oproj(u - 1)
            if u + 2 < UNITS:
                qk(u + 2, 1)
            if u + 1 < UNITS:
                softmax(u + 1)
        oproj(UNITS - 1)

    def step(it, carry):
        kv_wait(it)
        body(it)
        for r in range(2):
            @pl.when(jnp.logical_and(it + 2 < NIT, coords(it + 2)[1] == r))
            def _():
                start(kv_copies(it + 2, r))
        for j in range(NIT // NGP - 1):
            @pl.when(it == (j + 1) * NGP)
            def _():
                o_copy(j // 2, j % 2).start()
        return carry

    lax.fori_loop(0, NIT, step, 0)

    last_bg = B // NB - 1
    tail = [o_copy(last_bg, 1, 0, NTILE - DEFER), o_copy(last_bg, 1, NTILE - DEFER, NTILE)]
    tail[0].start()
    for t in range(NTILE - DEFER, NTILE):
        emit(NIT - 1, t, acc[t])
    tail[1].start()
    wait([o_copy(j // 2, j % 2) for j in range(NIT // NGP - 1)] + tail)


@jax.jit
def pallas_concat_heads__gqa_block_cached__gqa_block_cached__near_ridge_kernel(
    A_x: jax.Array,
    A_k_cache: jax.Array,
    A_v_cache: jax.Array,
    A_wq: jax.Array,
    A_wo: jax.Array,
    B_x: jax.Array,
    B_k_cache: jax.Array,
    B_v_cache: jax.Array,
    B_wq: jax.Array,
    B_wo: jax.Array,
):
    hbm = pl.BlockSpec(memory_space=pltpu.HBM)
    out = pl.pallas_call(
        _kernel,
        in_specs=[hbm] * 10,
        out_specs=hbm,
        out_shape=jax.ShapeDtypeStruct((B * SQ, 2 * D), BF16),
        scratch_shapes=[
            pltpu.VMEM((2, B * SQ, D), BF16),
            pltpu.VMEM((2, HKV, D, GW), BF16),
            pltpu.VMEM((2, NGP, D, NG * GW), BF16),
            pltpu.VMEM((HKV, 2, B, MQ // 2, DH), U32),
            pltpu.VMEM((2, 2, NB, NG, SK, DH), BF16),
            pltpu.VMEM((NTILE, D, TT), F32),
            pltpu.VMEM((NTILE, EDGE, TT), F32),
            pltpu.VMEM((2, B * SQ, WIN), BF16),
            pltpu.VMEM((MQ // 2, SK), U32),
            pltpu.VMEM((MQ // 2, SK), U32),
            pltpu.VMEM((TOK // 2, GW), U32),
            pltpu.VMEM((TOK // 2, GW), U32),
            pltpu.SemaphoreType.DMA((2,)),
            pltpu.SemaphoreType.DMA((6,)),
            pltpu.SemaphoreType.DMA((1,)),
        ],
        compiler_params=pltpu.CompilerParams(
            vmem_limit_bytes=120 * 1024 * 1024, disable_bounds_checks=True),
    )(A_x.reshape(B * SQ, D), A_k_cache, A_v_cache, A_wq, A_wo.T,
      B_x.reshape(B * SQ, D), B_k_cache, B_v_cache, B_wq, B_wo.T)
    return out.reshape(B, SQ, 2 * D)
```
